```python
import jax
import jax.numpy as jnp

def _softmax(x, axis=-1):
    return jax.nn.softmax(x, axis=axis)
def _gelu(x):
    return jax.nn.gelu(x, approximate=True)
def _silu(x):
    return jax.nn.silu(x)
def _sigmoid(x):
    return jax.nn.sigmoid(x)
def _layernorm(x, axis=-1, eps=1e-5):
    m = jnp.mean(x, axis=axis, keepdims=True)
    v = jnp.var(x, axis=axis, keepdims=True)
    return (x - m) / jnp.sqrt(v + eps)
def _scatter_add(tgt, idx, src, axis=0):
    return tgt.at[idx].add(src)
def _segment_sum(src, seg, n):
    return jax.ops.segment_sum(src, seg, n)
class _Rng:
    def __init__(self, key):
        self._k = key
    def _next(self):
        self._k, sub = jax.random.split(self._k)
        return sub
    def normal(self, shape):
        return jax.random.normal(self._next(), shape, dtype=jnp.bfloat16)
    def randint(self, lo, hi, shape):
        return jax.random.randint(self._next(), shape, lo, hi, dtype=jnp.int32)
    def uniform(self, shape, lo=0.0, hi=1.0):
        return jax.random.uniform(self._next(), shape, jnp.bfloat16, lo, hi)
    def permutation(self, n):
        return jax.random.permutation(self._next(), n)


kernel_name = 'concat_heads__compressed_kv_cla__gqa_block_cached__decode'

def setup_inputs():
    _rng = _Rng(jax.random.key(int.from_bytes(__import__("os").urandom(4), "little")))
    _w = (lambda a: (lambda t: t.astype(jnp.bfloat16) if jnp.issubdtype(t.dtype, jnp.floating) else t)(jnp.asarray(a)))
    def _A_setup():
        B, H, Sq, Sk, D, M = 2, 32, 1, 4096, 128, 512
        Dc = 4 * D
        return {
            "x": _w((lambda *s: _rng.normal(s) * 0.05)(B, Sq, M)),
            "c_kv": _w((lambda *s: _rng.normal(s) * 0.05)(B, Sk, Dc)),
            "w_q": _w((lambda *s: _rng.normal(s) * 0.05)(M, H, D) * (M ** -0.5)),
            "w_uk": _w((lambda *s: _rng.normal(s) * 0.05)(Dc, H, D) * (Dc ** -0.5)),
            "w_uv": _w((lambda *s: _rng.normal(s) * 0.05)(Dc, H, D) * (Dc ** -0.5)),
            "w_o": _w((lambda *s: _rng.normal(s) * 0.05)(H, D, M) * ((H * D) ** -0.5)),
        }
    _A_in = _A_setup()

    def _B_setup():
        B, Sq, D = 2, 1, 512
        Hq, Hkv, Sk, Dh = 32, 32, 4096, 128
        assert Hq % Hkv == 0, (Hq, Hkv)
        return {
            "x": _w((lambda *s: _rng.normal(s) * 0.05)(B, Sq, D)),
            "k_cache": _w((lambda *s: _rng.normal(s) * 0.05)(B, Hkv, Sk, Dh)),
            "v_cache": _w((lambda *s: _rng.normal(s) * 0.05)(B, Hkv, Sk, Dh)),
            "wq": _w((lambda *s: _rng.normal(s) * 0.05)(D, Hq * Dh) * (D ** -0.5)),
            "wo": _w((lambda *s: _rng.normal(s) * 0.05)(Hq * Dh, D) * ((Hq * Dh) ** -0.5)),
        }
    _B_in = _B_setup()

    return {
        "A_x": _A_in["x"],
        "A_c_kv": _A_in["c_kv"],
        "A_w_q": _A_in["w_q"],
        "A_w_uk": _A_in["w_uk"],
        "A_w_uv": _A_in["w_uv"],
        "A_w_o": _A_in["w_o"],
        "B_x": _B_in["x"],
        "B_k_cache": _B_in["k_cache"],
        "B_v_cache": _B_in["v_cache"],
        "B_wq": _B_in["wq"],
        "B_wo": _B_in["wo"],
    }

def reference(A_x, A_c_kv, A_w_q, A_w_uk, A_w_uv, A_w_o, B_x, B_k_cache, B_v_cache, B_wq, B_wo):
    def _A_ref(x, c_kv, w_q, w_uk, w_uv, w_o):
        B, Sq, M = x.shape[0], x.shape[1], x.shape[2]
        Sk = c_kv.shape[1]
        H, D = w_q.shape[1], w_q.shape[2]
        q = jnp.einsum("bqm,mhd->bhqd", x, w_q)
        k = jnp.einsum("bkc,chd->bhkd", c_kv, w_uk)
        v = jnp.einsum("bkc,chd->bhkd", c_kv, w_uv)
        scores = jnp.einsum("bhqd,bhkd->bhqk", q, k) * (D ** -0.5)
        off = Sk - Sq
        qi = jnp.arange(Sq)[:, None]
        kj = jnp.arange(Sk)[None, :]
        cmask = kj <= (qi + off)
        scores = jnp.where(cmask[None, None], scores, -1e9)
        p = _softmax(scores, axis=-1)
        ctx = jnp.einsum("bhqk,bhkd->bhqd", p, v)
        return jnp.einsum("bhqd,hdm->bqm", ctx, w_o)

    def _B_ref(x, k_cache, v_cache, wq, wo):
        B, Sq, D = x.shape
        Hq, Dh = 32, 128
        Hkv = k_cache.shape[1]
        rep = Hq // Hkv
        q = (lambda x, *d: x.transpose(*d))((x @ wq).reshape(B, Sq, Hq, Dh), 0, 2, 1, 3)
        k = jnp.repeat(k_cache, rep, axis=1)
        v = jnp.repeat(v_cache, rep, axis=1)
        scores = jnp.einsum("bhqd,bhkd->bhqk", q, k) * (Dh ** -0.5)
        p = _softmax(scores, axis=-1)
        o = jnp.einsum("bhqk,bhkd->bhqd", p, v)
        return (lambda x, *d: x.transpose(*d))(o, 0, 2, 1, 3).reshape(B, Sq, Hq * Dh) @ wo

    a = _A_ref(A_x, A_c_kv, A_w_q, A_w_uk, A_w_uv, A_w_o)
    b = _B_ref(B_x, B_k_cache, B_v_cache, B_wq, B_wo)
    return jnp.concatenate([a, b], axis=-1)
```

```python
import jax
import jax.numpy as jnp
from jax import lax
import jax.experimental.pallas as pl
import jax.experimental.pallas.tpu as pltpu

F32 = jnp.float32
BF16 = jnp.bfloat16
NT = (((1,), (1,)), ((), ()))

G = 8
KV_ROWS = 64
KV_LEAD = 16


def _kernel(ax_hbm, ckv_hbm, wq_hbm, wuk_hbm, wuv_hbm, wo_hbm,
            bx_hbm, k_hbm, v_hbm, bwq_hbm, bwo_hbm,
            out_hbm,
            ax, ckv, wq, wuk, wuv, wo, bx, kbuf, vbuf, bwq, bwo,
            qb_ref, qa_ref, sa_ref, pa_ref, cl_ref, ctx_ref, ob_ref, s_ref, p_ref,
            out_ref, x_sem, w_sem, kv_sem, o_sem, out_sem):
    n_pairs, sk, dh = k_hbm.shape
    n_chunks = n_pairs // G
    n_blk = sk // KV_ROWS
    nq, q_rows, _ = wq.shape
    heads = 32
    n_u = heads // 8
    sm_scale = dh ** -0.5

    def copy(src, dst, idx, sem, priority):
        pltpu.make_async_copy(src.at[idx], dst.at[idx], sem).start(priority=priority)

    def wait_all(buf, sem):
        pltpu.make_async_copy(buf, buf, sem).wait()

    def start_tall(src, dst, sem, i):
        rows = pl.ds(pl.multiple_of(i * 64, 64), 64)
        copy(src, dst, (pl.ds(0, 2), rows), sem, 0)
        copy(src, dst, (pl.ds(2, 2), rows), sem, 1)

    def start_wide(src, dst, sem, i, n_streams):
        rows = pl.ds(pl.multiple_of(i * 16, 16), 16)
        for g in range(n_streams // 2):
            copy(src, dst, (pl.ds(2 * g, 2), rows), sem, g % 2)

    def start_bwq(sem, i):
        rows = pl.ds(pl.multiple_of((i // 8) * 16, 16), 16)
        cols = pl.ds(pl.multiple_of((i % 8) * 512, 512), 512)
        copy(bwq_hbm, bwq, (pl.ds(0, 2), rows, cols), sem, 0)
        copy(bwq_hbm, bwq, (pl.ds(2, 2), rows, cols), sem, 1)

    def start_first(i):
        start_bwq(w_sem.at[0], i)
        start_tall(wq_hbm, wq, w_sem.at[1], i)
        start_tall(wuk_hbm, wuk, w_sem.at[2], i)

    def start_second(i):
        start_wide(ckv_hbm, ckv, w_sem.at[3], i, ckv.shape[0])
        start_tall(wuv_hbm, wuv, w_sem.at[4], i)

    def start_kv(t, i):
        slot = t % 2
        rows = pl.ds(pl.multiple_of(i * KV_ROWS, KV_ROWS), KV_ROWS)
        for g in range(G // 2):
            for src, dst, a in ((k_hbm, kbuf, 0), (v_hbm, vbuf, 1)):
                pltpu.make_async_copy(
                    src.at[pl.ds(t * G + 2 * g, 2), rows],
                    dst.at[slot, pl.ds(2 * g, 2), rows],
                    kv_sem.at[a, slot],
                ).start(priority=a)

    n_slices = o_sem.shape[0]
    blk_per_slice = 64 // n_slices

    def start_last(i):
        sem = o_sem.at[i // blk_per_slice]
        start_wide(wo_hbm, wo, sem, i, wo.shape[0])
        start_wide(bwo_hbm, bwo, sem, i, bwo.shape[0])

    def issue(start_fn, lo, n):
        def body(i, _):
            start_fn(lo + i)
        lax.fori_loop(0, n, body, None)

    def rows16(x_ref):
        x = x_ref[...].astype(F32)
        shape = (16, x.shape[1])
        r = lax.broadcasted_iota(jnp.int32, shape, 0)
        return jnp.where(r < 8, jnp.broadcast_to(x[0:1], shape),
                         jnp.broadcast_to(x[1:2], shape)).astype(BF16)

    def row_is(j, shape):
        return (lax.broadcasted_iota(jnp.int32, shape, 0) & 7) == j

    def head_pair(w_ref, u, jj):
        stride = heads // 2
        n = q_rows // heads
        words = w_ref.bitcast(jnp.uint32).at[
            :, pl.ds(pl.multiple_of(4 * u, 4), (n - 1) * stride + 4), :]
        x = words[:, pl.ds(jj, n, stride=stride), :].reshape(nq * n, dh)
        even = pltpu.bitcast(x << 16, F32).astype(BF16)
        odd = pltpu.bitcast(x & jnp.uint32(0xFFFF0000), F32).astype(BF16)
        return even, odd

    def softmax_parts(s):
        s = s * sm_scale
        p = jnp.exp(s - jnp.max(s, axis=1, keepdims=True))
        return p.astype(BF16), jnp.sum(p, axis=1, keepdims=True)

    start_first(0)
    ax_copy = pltpu.make_async_copy(ax_hbm, ax, x_sem.at[0])
    bx_copy = pltpu.make_async_copy(bx_hbm, bx, x_sem.at[1])
    ax_copy.start()
    bx_copy.start()
    issue(start_first, 1, 63)
    s_ref[...] = jnp.zeros(s_ref.shape, F32)
    issue(start_second, 0, 16)

    ax_copy.wait()
    bx_copy.wait()
    wait_all(bwq, w_sem.at[0])
    wait_all(wq, w_sem.at[1])
    wait_all(wuk, w_sem.at[2])

    xb = rows16(bx)
    xa = rows16(ax)

    for u in range(n_u):
        cols = slice(u * 8 * dh, (u + 1) * 8 * dh)
        r = None
        for qd in range(bwq.shape[0]):
            d = jnp.dot(xb[:, qd * 128:(qd + 1) * 128], bwq[qd, :, cols],
                        preferred_element_type=F32)
            r = d if r is None else r + d
        q = jnp.zeros((16, dh), F32)
        for j in range(8):
            q = jnp.where(row_is(j, (16, dh)), r[:, j * dh:(j + 1) * dh], q)
        qb_ref[u] = q
        issue(start_second, 16 + 4 * u, 4)

    def absorb_group(u, _):
        acc = jnp.zeros((16, ckv.shape[2]), F32)
        for jj in range(4):
            q_pair = head_pair(wq, u, jj)
            k_pair = head_pair(wuk, u, jj)
            for e in range(2):
                q = jnp.dot(xa, q_pair[e], preferred_element_type=F32).astype(BF16)
                qa = lax.dot_general(q, k_pair[e], NT, preferred_element_type=F32)
                acc = jnp.where(row_is(2 * jj + e, acc.shape), qa, acc)
            issue(start_second, 32 + (u * 4 + jj) * 2, 2)
        rows = pl.ds(pl.multiple_of(u * 8, 8), 8)
        qa_ref[0, rows, :] = acc[0:8]
        qa_ref[1, rows, :] = acc[8:16]
    lax.fori_loop(0, n_u, absorb_group, None)

    issue(lambda i: start_kv(0, i), 0, KV_LEAD)
    wait_all(ckv, w_sem.at[3])
    wait_all(wuv, w_sem.at[4])

    parts = ckv.shape[0] // 2

    def latent(b, _):
        base = KV_LEAD + b * 16
        qa = qa_ref[b].astype(BF16)

        def scores(c, _):
            sa_ref[c] = lax.dot_general(qa, ckv[b * parts + c], NT,
                                        preferred_element_type=F32) * sm_scale
            issue(lambda i: start_kv(0, i), base + 2 * c, 2)
        lax.fori_loop(0, parts, scores, None)

        m = jnp.max(sa_ref[0], axis=1, keepdims=True)
        for c in range(1, parts):
            m = jnp.maximum(m, jnp.max(sa_ref[c], axis=1, keepdims=True))
        l = jnp.zeros_like(m)
        for c in range(parts):
            p = jnp.exp(sa_ref[c] - m)
            l = l + jnp.sum(p, axis=1, keepdims=True)
            pa_ref[c] = p.astype(BF16)

        def context(c, acc):
            acc = acc + jnp.dot(pa_ref[c], ckv[b * parts + c], preferred_element_type=F32)
            issue(lambda i: start_kv(0, i), base + 8 + 2 * c, 2)
            return acc
        acc = lax.fori_loop(0, parts, context, jnp.zeros((heads, ckv.shape[2]), F32))
        acc = acc / l
        rows = pl.ds(pl.multiple_of(b * 8, 8), 8)
        for u in range(n_u):
            cl_ref[u, rows, :] = acc[u * 8:(u + 1) * 8]
    lax.fori_loop(0, 2, latent, None)

    def up_group(u, _):
        cl = cl_ref[u].astype(BF16)

        acc = jnp.zeros((16, dh), F32)
        for jj in range(4):
            v_pair = head_pair(wuv, u, jj)
            for e in range(2):
                r = jnp.dot(cl, v_pair[e], preferred_element_type=F32)
                acc = jnp.where(row_is(2 * jj + e, acc.shape), r, acc)
            issue(lambda i: start_kv(0, i), KV_LEAD + 32 + u * 4 + jj, 1)
        ctx_ref[u] = acc
    lax.fori_loop(0, n_u, up_group, None)

    per_step = (n_blk - KV_LEAD) // (2 * G)

    def attend(t, start_next):
        slot = t % 2
        issue(start_next, 0, KV_LEAD)
        wait_all(kbuf.at[slot], kv_sem.at[0, slot])
        wait_all(vbuf.at[slot], kv_sem.at[1, slot])
        u = t % n_u
        rows = pl.ds(pl.multiple_of((t // n_u) * 8, 8), 8)
        q = qb_ref[u, rows, :].astype(BF16)

        def scores(j, _):
            s = lax.dot_general(q, kbuf[slot, j], NT, preferred_element_type=F32)
            s_ref[...] = jnp.where(row_is(j, s.shape), s, s_ref[...])
            issue(start_next, KV_LEAD + j * per_step, per_step)
        lax.fori_loop(0, G, scores, None)

        p, l = softmax_parts(s_ref[...])
        p_ref[...] = p

        def values(j, acc):
            r = jnp.dot(p_ref[...], vbuf[slot, j], preferred_element_type=F32)
            issue(start_next, KV_LEAD + (G + j) * per_step, per_step)
            return jnp.where(row_is(j, r.shape), r, acc)
        o = lax.fori_loop(0, G, values, jnp.zeros((G, dh), F32))
        ob_ref[u, rows, :] = o / l

    def attend_and_fetch(t, _):
        attend(t, lambda i: start_kv(t + 1, i))
    lax.fori_loop(0, n_chunks - 1, attend_and_fetch, None)
    attend(n_chunks - 1, start_last)

    heads_per_slice = 8 // n_slices

    def project(i, accs):
        acc_a, acc_b = accs
        rows = pl.ds(pl.multiple_of(i * heads_per_slice * dh, dh), heads_per_slice * dh)
        wait_all(wo.at[:, rows], o_sem.at[i])
        wait_all(bwo.at[:, rows], o_sem.at[i])
        for e in range(heads_per_slice):
            j = i * heads_per_slice + e
            keep = row_is(j, (16, dh))
            hrows = pl.ds(pl.multiple_of(j * dh, dh), dh)
            for u in range(n_u):
                lhs = jnp.where(keep, ctx_ref[u], 0.0).astype(BF16)
                acc_a = acc_a + jnp.dot(lhs, wo[u, hrows, :], preferred_element_type=F32)
                lhs = jnp.where(keep, ob_ref[u], 0.0).astype(BF16)
                acc_b = acc_b + jnp.dot(lhs, bwo[u, hrows, :], preferred_element_type=F32)
        return acc_a, acc_b

    zero = jnp.zeros((16, wo.shape[2]), F32)
    acc_a, acc_b = lax.fori_loop(0, n_slices, project, (zero, zero))
    acc = jnp.concatenate([acc_a, acc_b], axis=1)
    first = jnp.sum(acc[0:8], axis=0, keepdims=True)
    second = jnp.sum(acc[8:16], axis=0, keepdims=True)
    r = lax.broadcasted_iota(jnp.int32, out_ref.shape, 0)
    out_ref[...] = jnp.where(r == 0, first, second).astype(out_ref.dtype)
    out_copy = pltpu.make_async_copy(out_ref, out_hbm, out_sem)
    out_copy.start()
    out_copy.wait()


@jax.jit
def pallas_concat_heads__compressed_kv_cla__gqa_block_cached__decode_kernel(
    A_x: jax.Array,
    A_c_kv: jax.Array,
    A_w_q: jax.Array,
    A_w_uk: jax.Array,
    A_w_uv: jax.Array,
    A_w_o: jax.Array,
    B_x: jax.Array,
    B_k_cache: jax.Array,
    B_v_cache: jax.Array,
    B_wq: jax.Array,
    B_wo: jax.Array,
):
    B, Sq, M = A_x.shape
    _, Sk, Dc = A_c_kv.shape
    _, H, D = A_w_q.shape
    _, Hkv, SkB, Dh = B_k_cache.shape
    MB = B_x.shape[2]
    assert (B, Sq, M, Sk, Dc, H, D) == (2, 1, 512, 4096, 512, 32, 128)
    assert (Hkv, SkB, Dh, MB) == (32, 4096, 128, 512)

    args = (
        A_x.reshape(B, M),
        A_c_kv.reshape(8, 1024, Dc),
        A_w_q.reshape(4, M * H // 4, D),
        A_w_uk.reshape(4, Dc * H // 4, D),
        A_w_uv.reshape(4, Dc * H // 4, D),
        A_w_o.reshape(4, H * D // 4, M),
        B_x.reshape(B, MB),
        B_k_cache.reshape(B * Hkv, SkB, Dh),
        B_v_cache.reshape(B * Hkv, SkB, Dh),
        B_wq.reshape(4, MB // 4, Hkv * Dh),
        B_wo.reshape(4, Hkv * Dh // 4, MB),
    )

    def like(x):
        return pltpu.VMEM(x.shape, x.dtype)

    scratch = [
        like(args[0]), like(args[1]), like(args[2]), like(args[3]), like(args[4]),
        like(args[5]), like(args[6]),
        pltpu.VMEM((2, G, SkB, Dh), BF16),
        pltpu.VMEM((2, G, SkB, Dh), BF16),
        like(args[9]), like(args[10]),
        pltpu.VMEM((H // 8, 16, Dh), F32),
        pltpu.VMEM((B, H, Dc), F32),
        pltpu.VMEM((4, H, 1024), F32),
        pltpu.VMEM((4, H, 1024), BF16),
        pltpu.VMEM((H // 8, 16, Dc), F32),
        pltpu.VMEM((H // 8, 16, D), F32),
        pltpu.VMEM((H // 8, 16, Dh), F32),
        pltpu.VMEM((G, SkB), F32),
        pltpu.VMEM((G, SkB), BF16),
        pltpu.VMEM((B, M + MB), BF16),
        pltpu.SemaphoreType.DMA((2,)),
        pltpu.SemaphoreType.DMA((5,)),
        pltpu.SemaphoreType.DMA((2, 2)),
        pltpu.SemaphoreType.DMA((8,)),
        pltpu.SemaphoreType.DMA(()),
    ]
    out = pl.pallas_call(
        _kernel,
        in_specs=[pl.BlockSpec(memory_space=pltpu.HBM)] * len(args),
        out_specs=pl.BlockSpec(memory_space=pltpu.HBM),
        out_shape=jax.ShapeDtypeStruct((B, M + MB), BF16),
        scratch_shapes=scratch,
        compiler_params=pltpu.CompilerParams(vmem_limit_bytes=100 * 1024 * 1024),
    )(*args)
    return out.reshape(B, Sq, M + MB)
```

```python
import jax
import jax.numpy as jnp
from jax import lax
import jax.experimental.pallas as pl
import jax.experimental.pallas.tpu as pltpu

F32 = jnp.float32
BF16 = jnp.bfloat16
NT = (((1,), (1,)), ((), ()))

G = 8
KV_ROWS = 64
SPLIT = 5
KV_LEAD = 16


def _kernel(ax_hbm, ckv_hbm, wq_hbm, wuk_hbm, wuv_hbm, wo_hbm,
            bx_hbm, k_hbm, v_hbm, bwq_hbm, bwo_hbm,
            out_hbm,
            ax, ckv, wq, wuk, wuv, wo, bx, kv, bwq, bwo,
            qb_ref, qa_ref, sa_ref, pa_ref, cl_ref, ctx_ref, ob_ref, s_ref, p_ref,
            out_ref, sems):
    n_pairs, sk, dh = k_hbm.shape
    n_chunks = n_pairs // G
    n_blk = sk // KV_ROWS
    nq, q_rows, _ = wq.shape
    heads = 32
    n_u = heads // 8
    sm_scale = dh ** -0.5

    def copy(src, dst, idx, sem, priority):
        pltpu.make_async_copy(src.at[idx], dst.at[idx], sem).start(priority=priority)

    def wait_all(buf, sem):
        pltpu.make_async_copy(buf, buf, sem).wait()

    def start_tall(src, dst, sem, i, pair, priority):
        rows = pl.ds(pl.multiple_of(i * 64, 64), 64)
        copy(src, dst, (pl.ds(2 * pair, 2), rows), sem, priority)

    def start_wide(src, dst, sem, i, pair, priority):
        rows = pl.ds(pl.multiple_of(i * 16, 16), 16)
        copy(src, dst, (pl.ds(2 * pair, 2), rows), sem, priority)

    def start_flat(src, dst, sem, i, pair, priority):
        rows = pl.ds(pl.multiple_of((i // 4) * 8, 8), 8)
        cols = pl.ds(pl.multiple_of((i % 4) * 1024, 1024), 1024)
        copy(src, dst, (pl.ds(2 * pair, 2), rows, cols), sem, priority)

    def start_first(i):
        for g, (src, dst) in enumerate(((wq_hbm, wq), (wuk_hbm, wuk))):
            for pair in range(2):
                start_tall(src, dst, sems.at[0], i, pair, 0)
                start_wide(ckv_hbm, ckv, sems.at[0], i, 2 * g + pair, 1)

    def start_second(i):
        for pair in range(2):
            start_flat(bwq_hbm, bwq, sems.at[1], i, pair, 0)
            start_tall(wuv_hbm, wuv, sems.at[1], i, pair, 1)

    def start_kv(t, i):
        slot = t % 2
        rows = pl.ds(pl.multiple_of(i * KV_ROWS, KV_ROWS), KV_ROWS)
        for g in range(G // 2):
            for a, src in enumerate((k_hbm, v_hbm)):
                pltpu.make_async_copy(
                    src.at[pl.ds(t * G + 2 * g, 2), rows],
                    kv.at[slot, a, pl.ds(2 * g, 2), rows],
                    sems.at[slot],
                ).start(priority=a)

    def start_kv0(i):
        start_kv(0, i)

    def start_last(i):
        sem = sems.at[(i >= 8 * SPLIT).astype(jnp.int32)]
        for pair in range(2):
            start_wide(wo_hbm, wo, sem, i, pair, 0)
            start_wide(bwo_hbm, bwo, sem, i, pair, 1)

    def start_tail_head(i):
        for e in range(2):
            blk = 56 + 2 * i + e
            start_wide(wo_hbm, wo, sems.at[2], blk, 0, e)
            start_wide(wo_hbm, wo, sems.at[2], blk, 1, 1 - e)
            start_wide(bwo_hbm, bwo, sems.at[2], blk, 0, e)

    def start_tail_end(i):
        for e in range(2):
            start_wide(bwo_hbm, bwo, sems.at[3], 56 + 2 * i + e, 1, e)

    def issue(start_fn, lo, n):
        def body(i, _):
            start_fn(lo + i)
        lax.fori_loop(0, n, body, None)

    def rows16(x_ref):
        x = x_ref[...].astype(F32)
        shape = (16, x.shape[1])
        r = lax.broadcasted_iota(jnp.int32, shape, 0)
        return jnp.where(r < 8, jnp.broadcast_to(x[0:1], shape),
                         jnp.broadcast_to(x[1:2], shape)).astype(BF16)

    def row_is(j, shape):
        return (lax.broadcasted_iota(jnp.int32, shape, 0) & 7) == j

    def head_pair(w_ref, u, jj):
        stride = heads // 2
        n = q_rows // heads
        words = w_ref.bitcast(jnp.uint32).at[
            :, pl.ds(pl.multiple_of(4 * u, 4), (n - 1) * stride + 4), :]
        x = words[:, pl.ds(jj, n, stride=stride), :].reshape(nq * n, dh)
        even = pltpu.bitcast(x << 16, F32).astype(BF16)
        odd = pltpu.bitcast(x & jnp.uint32(0xFFFF0000), F32).astype(BF16)
        return even, odd

    def softmax_parts(s):
        s = s * sm_scale
        p = jnp.exp(s - jnp.max(s, axis=1, keepdims=True))
        return p.astype(BF16), jnp.sum(p, axis=1, keepdims=True)

    start_first(0)
    ax_copy = pltpu.make_async_copy(ax_hbm, ax, sems.at[0])
    bx_copy = pltpu.make_async_copy(bx_hbm, bx, sems.at[0])
    ax_copy.start()
    bx_copy.start()
    issue(start_first, 1, 63)
    s_ref[...] = jnp.zeros(s_ref.shape, F32)
    issue(start_second, 0, 16)

    ax_copy.wait()
    bx_copy.wait()
    wait_all(wq, sems.at[0])
    wait_all(wuk, sems.at[0])
    wait_all(ckv, sems.at[0])

    xa = rows16(ax)

    def absorb_group(u, _):
        acc = jnp.zeros((16, ckv.shape[2]), F32)
        for jj in range(4):
            q_pair = head_pair(wq, u, jj)
            k_pair = head_pair(wuk, u, jj)
            for e in range(2):
                q = jnp.dot(xa, q_pair[e], preferred_element_type=F32).astype(BF16)
                qa = lax.dot_general(q, k_pair[e], NT, preferred_element_type=F32)
                acc = jnp.where(row_is(2 * jj + e, acc.shape), qa, acc)
            pl.when(u < 2)(lambda: issue(start_second, 16 + (u * 4 + jj) * 6, 6))
            pl.when(u >= 2)(lambda: issue(start_kv0, ((u - 2) * 4 + jj) * 3, 3))
        rows = pl.ds(pl.multiple_of(u * 8, 8), 8)
        qa_ref[0, rows, :] = acc[0:8]
        qa_ref[1, rows, :] = acc[8:16]
    lax.fori_loop(0, n_u, absorb_group, None)

    parts = ckv.shape[0] // 2

    def latent(b, _):
        base = 24 + b * 20
        qa = qa_ref[b].astype(BF16)

        def scores(c, _):
            sa_ref[c] = lax.dot_general(qa, ckv[b * parts + c], NT,
                                        preferred_element_type=F32) * sm_scale
            issue(start_kv0, base + 3 * c, 3)
        lax.fori_loop(0, parts, scores, None)

        m = jnp.max(sa_ref[0], axis=1, keepdims=True)
        for c in range(1, parts):
            m = jnp.maximum(m, jnp.max(sa_ref[c], axis=1, keepdims=True))
        l = jnp.zeros_like(m)
        for c in range(parts):
            p = jnp.exp(sa_ref[c] - m)
            l = l + jnp.sum(p, axis=1, keepdims=True)
            pa_ref[c] = p.astype(BF16)

        def context(c, acc):
            acc = acc + jnp.dot(pa_ref[c], ckv[b * parts + c], preferred_element_type=F32)
            issue(start_kv0, base + 12 + 2 * c, 2)
            return acc
        acc = lax.fori_loop(0, parts, context, jnp.zeros((heads, ckv.shape[2]), F32))
        acc = acc / l
        rows = pl.ds(pl.multiple_of(b * 8, 8), 8)
        for u in range(n_u):
            cl_ref[u, rows, :] = acc[u * 8:(u + 1) * 8]
    lax.fori_loop(0, 2, latent, None)

    wait_all(bwq, sems.at[1])
    wait_all(wuv, sems.at[1])

    def up_project(u):
        cl = cl_ref[u].astype(BF16)
        acc = jnp.zeros((16, dh), F32)
        for jj in range(4):
            v_pair = head_pair(wuv, u, jj)
            for e in range(2):
                r = jnp.dot(cl, v_pair[e], preferred_element_type=F32)
                acc = jnp.where(row_is(2 * jj + e, acc.shape), r, acc)
        ctx_ref[u] = acc

    def queries(u):
        xb = rows16(bx)
        cols = pl.ds(pl.multiple_of(u * 8 * dh, 8 * dh), 8 * dh)
        r = None
        for qd in range(bwq.shape[0]):
            d = jnp.dot(xb[:, qd * 128:(qd + 1) * 128], bwq[qd, :, cols],
                        preferred_element_type=F32)
            r = d if r is None else r + d
        q = jnp.zeros((16, dh), F32)
        for j in range(8):
            q = jnp.where(row_is(j, (16, dh)), r[:, j * dh:(j + 1) * dh], q)
        qb_ref[u] = q

    def attend(t, start_next, lead, per_step):
        slot = t % 2
        issue(start_next, 0, lead)
        if not isinstance(t, int):
            @pl.when(t < n_u)
            def _():
                up_project(t)
                queries(t)
        wait_all(kv.at[slot], sems.at[slot])
        u = t % n_u
        rows = pl.ds(pl.multiple_of((t // n_u) * 8, 8), 8)
        q = qb_ref[u, rows, :].astype(BF16)

        def scores(j, _):
            s = lax.dot_general(q, kv[slot, 0, j], NT, preferred_element_type=F32)
            s_ref[...] = jnp.where(row_is(j, s.shape), s, s_ref[...])
            issue(start_next, lead + j * per_step, per_step)
        lax.fori_loop(0, G, scores, None)

        p, l = softmax_parts(s_ref[...])
        p_ref[...] = p

        def values(j, acc):
            r = jnp.dot(p_ref[...], kv[slot, 1, j], preferred_element_type=F32)
            issue(start_next, lead + (G + j) * per_step, per_step)
            return jnp.where(row_is(j, r.shape), r, acc)
        o = lax.fori_loop(0, G, values, jnp.zeros((G, dh), F32))
        ob_ref[u, rows, :] = o / l

    def attend_and_fetch(t, _):
        attend(t, lambda i: start_kv(t + 1, i), KV_LEAD, (n_blk - KV_LEAD) // (2 * G))
    lax.fori_loop(0, n_chunks - 1, attend_and_fetch, None)
    attend(n_chunks - 1, start_last, 24, 2)
    issue(start_tail_head, 0, 4)
    issue(start_tail_end, 0, 4)

    def head_rows(o_ref, u, j):
        r = lax.broadcasted_iota(jnp.int32, (8, dh), 0)
        return jnp.where(
            r == 0,
            jnp.broadcast_to(o_ref[u, pl.ds(j, 1), :], (8, dh)),
            jnp.broadcast_to(o_ref[u, pl.ds(8 + j, 1), :], (8, dh))).astype(BF16)

    def add_heads(acc, lhs, w_ref, groups, j):
        hrows = pl.ds(pl.multiple_of(j * dh, dh), dh)
        for x, u in zip(lhs, groups):
            acc = acc + jnp.dot(x, w_ref[u, hrows, :], preferred_element_type=F32)
        return acc

    def project(j, accs):
        groups = range(n_u)
        return (
            add_heads(accs[0], [head_rows(ctx_ref, u, j) for u in groups], wo, groups, j),
            add_heads(accs[1], [head_rows(ob_ref, u, j) for u in groups], bwo, groups, j))

    zero = jnp.zeros((8, wo.shape[2]), F32)
    accs = (zero, zero)
    for piece, (lo, hi) in enumerate(((0, SPLIT), (SPLIT, 7))):
        rows = pl.ds(lo * dh, (hi - lo) * dh)
        wait_all(wo.at[:, rows], sems.at[piece])
        wait_all(bwo.at[:, rows], sems.at[piece])
        accs = lax.fori_loop(lo, hi, project, accs)
    acc_a, acc_b = accs

    rows = pl.ds(7 * dh, dh)
    lhs_a = [head_rows(ctx_ref, u, 7) for u in range(n_u)]
    lhs_b = [head_rows(ob_ref, u, 7) for u in range(n_u)]
    wait_all(wo.at[:, rows], sems.at[2])
    wait_all(bwo.at[0:2, rows], sems.at[2])
    acc_a = add_heads(acc_a, lhs_a, wo, range(n_u), 7)
    acc_b = add_heads(acc_b, lhs_b[:2], bwo, (0, 1), 7)
    out_ref[:, :wo.shape[2]] = acc_a[0:2].astype(out_ref.dtype)
    wait_all(bwo.at[2:4, rows], sems.at[3])
    acc_b = add_heads(acc_b, lhs_b[2:], bwo, (2, 3), 7)
    out_ref[:, wo.shape[2]:] = acc_b[0:2].astype(out_ref.dtype)
    out_copy = pltpu.make_async_copy(out_ref, out_hbm, sems.at[0])
    out_copy.start()
    out_copy.wait()


@jax.jit
def pallas_concat_heads__compressed_kv_cla__gqa_block_cached__decode_kernel(
    A_x: jax.Array,
    A_c_kv: jax.Array,
    A_w_q: jax.Array,
    A_w_uk: jax.Array,
    A_w_uv: jax.Array,
    A_w_o: jax.Array,
    B_x: jax.Array,
    B_k_cache: jax.Array,
    B_v_cache: jax.Array,
    B_wq: jax.Array,
    B_wo: jax.Array,
):
    B, Sq, M = A_x.shape
    _, Sk, Dc = A_c_kv.shape
    _, H, D = A_w_q.shape
    _, Hkv, SkB, Dh = B_k_cache.shape
    MB = B_x.shape[2]
    assert (B, Sq, M, Sk, Dc, H, D) == (2, 1, 512, 4096, 512, 32, 128)
    assert (Hkv, SkB, Dh, MB) == (32, 4096, 128, 512)

    args = (
        A_x.reshape(B, M),
        A_c_kv.reshape(8, 1024, Dc),
        A_w_q.reshape(4, M * H // 4, D),
        A_w_uk.reshape(4, Dc * H // 4, D),
        A_w_uv.reshape(4, Dc * H // 4, D),
        A_w_o.reshape(4, H * D // 4, M),
        B_x.reshape(B, MB),
        B_k_cache.reshape(B * Hkv, SkB, Dh),
        B_v_cache.reshape(B * Hkv, SkB, Dh),
        B_wq.reshape(4, MB // 4, Hkv * Dh),
        B_wo.reshape(4, Hkv * Dh // 4, MB),
    )

    def like(x):
        return pltpu.VMEM(x.shape, x.dtype)

    scratch = [
        like(args[0]), like(args[1]), like(args[2]), like(args[3]), like(args[4]),
        like(args[5]), like(args[6]),
        pltpu.VMEM((2, 2, G, SkB, Dh), BF16),
        like(args[9]), like(args[10]),
        pltpu.VMEM((H // 8, 16, Dh), F32),
        pltpu.VMEM((B, H, Dc), F32),
        pltpu.VMEM((4, H, 1024), F32),
        pltpu.VMEM((4, H, 1024), BF16),
        pltpu.VMEM((H // 8, 16, Dc), F32),
        pltpu.VMEM((H // 8, 16, D), F32),
        pltpu.VMEM((H // 8, 16, Dh), F32),
        pltpu.VMEM((G, SkB), F32),
        pltpu.VMEM((G, SkB), BF16),
        pltpu.VMEM((B, M + MB), BF16),
        pltpu.SemaphoreType.DMA((4,)),
    ]
    out = pl.pallas_call(
        _kernel,
        in_specs=[pl.BlockSpec(memory_space=pltpu.HBM)] * len(args),
        out_specs=pl.BlockSpec(memory_space=pltpu.HBM),
        out_shape=jax.ShapeDtypeStruct((B, M + MB), BF16),
        scratch_shapes=scratch,
        compiler_params=pltpu.CompilerParams(vmem_limit_bytes=100 * 1024 * 1024),
    )(*args)
    return out.reshape(B, Sq, M + MB)
```

```python
import jax
import jax.numpy as jnp
from jax import lax
import jax.experimental.pallas as pl
import jax.experimental.pallas.tpu as pltpu

F32 = jnp.float32
BF16 = jnp.bfloat16
NT = (((1,), (1,)), ((), ()))

G = 8
BLOCKS = 64
LEAD = 16
SPLIT = 5


def _kernel(ax_hbm, ckv_hbm, wq_hbm, wuk_hbm, wuv_hbm, wo_hbm,
            bx_hbm, k_hbm, v_hbm, bwq_hbm, bwo_hbm,
            out_hbm,
            ax, ckv, wq, wuk, wuv, wo, bx, kv, bwq, bwo,
            qb_ref, qa_ref, sa_ref, pa_ref, cl_ref, ctx_ref, ob_ref, s_ref, p_ref,
            out_ref, sems):
    n_pairs, _, dh = k_hbm.shape
    n_chunks = n_pairs // G
    n_slabs, slab_rows, _ = wq.shape
    heads = qa_ref.shape[1]
    n_u = heads // 8
    dc = ckv.shape[2]
    sm_scale = dh ** -0.5

    def copy(src, dst, idx, sem, queue):
        pltpu.make_async_copy(src.at[idx], dst.at[idx], sem).start(priority=queue)

    def wait_for(buf, sem):
        pltpu.make_async_copy(buf, buf, sem).wait()

    def start_tall(src, dst, sem, i, pair, queue):
        rows = pl.ds(pl.multiple_of(i * 64, 64), 64)
        copy(src, dst, (pl.ds(2 * pair, 2), rows), sem, queue)

    def start_wide(src, dst, sem, i, pair, queue):
        rows = pl.ds(pl.multiple_of(i * 16, 16), 16)
        copy(src, dst, (pl.ds(2 * pair, 2), rows), sem, queue)

    def start_flat(src, dst, sem, i, pair, queue):
        rows = pl.ds(pl.multiple_of((i // 4) * 8, 8), 8)
        cols = pl.ds(pl.multiple_of((i % 4) * 1024, 1024), 1024)
        copy(src, dst, (pl.ds(2 * pair, 2), rows, cols), sem, queue)

    def start_first(i):
        for g, (src, dst) in enumerate(((wq_hbm, wq), (wuk_hbm, wuk))):
            for pair in range(2):
                start_tall(src, dst, sems.at[0], i, pair, 0)
                start_wide(ckv_hbm, ckv, sems.at[0], i, 2 * g + pair, 1)

    def start_second(i):
        for pair in range(2):
            start_flat(bwq_hbm, bwq, sems.at[1], i, pair, 0)
            start_tall(wuv_hbm, wuv, sems.at[1], i, pair, 1)

    def start_chunk(t, i):
        slot = t % 2
        rows = pl.ds(pl.multiple_of(i * 64, 64), 64)
        for pair in range(G // 2):
            for a, src in enumerate((k_hbm, v_hbm)):
                pltpu.make_async_copy(
                    src.at[pl.ds(t * G + 2 * pair, 2), rows],
                    kv.at[slot, a, pl.ds(2 * pair, 2), rows],
                    sems.at[slot],
                ).start(priority=a)

    def start_chunk0(i):
        start_chunk(0, i)

    def start_last(i):
        sem = sems.at[(i >= 8 * SPLIT).astype(jnp.int32)]
        for pair in range(2):
            start_wide(wo_hbm, wo, sem, i, pair, 0)
            start_wide(bwo_hbm, bwo, sem, i, pair, 1)

    def start_tail(i):
        start_wide(wo_hbm, wo, sems.at[2], i, 0, 1)
        start_wide(wo_hbm, wo, sems.at[2], i, 1, 1)
        start_wide(bwo_hbm, bwo, sems.at[2], i, 0, 1)

    def start_end(i):
        start_wide(bwo_hbm, bwo, sems.at[3], i, 1, 1)

    def issue(start, first_block, n_blocks):
        def body(i, _):
            start(first_block + i)
        lax.fori_loop(0, n_blocks, body, None)

    def rows16(x_ref):
        x = x_ref[...].astype(F32)
        shape = (16, x.shape[1])
        r = lax.broadcasted_iota(jnp.int32, shape, 0)
        return jnp.where(r < 8, jnp.broadcast_to(x[0:1], shape),
                         jnp.broadcast_to(x[1:2], shape)).astype(BF16)

    def put_row(j, new, old):
        r = lax.broadcasted_iota(jnp.int32, new.shape, 0)
        return jnp.where((r & 7) == j, new, old)

    def head_pair(w_ref, u, jj):
        stride = heads // 2
        n = slab_rows // heads
        words = w_ref.bitcast(jnp.uint32).at[
            :, pl.ds(pl.multiple_of(4 * u, 4), (n - 1) * stride + 4), :]
        x = words[:, pl.ds(jj, n, stride=stride), :].reshape(n_slabs * n, dh)
        return (pltpu.bitcast(x << 16, F32).astype(BF16),
                pltpu.bitcast(x & jnp.uint32(0xFFFF0000), F32).astype(BF16))

    start_first(0)
    ax_copy = pltpu.make_async_copy(ax_hbm, ax, sems.at[2])
    bx_copy = pltpu.make_async_copy(bx_hbm, bx, sems.at[3])
    ax_copy.start()
    bx_copy.start()
    issue(start_first, 1, BLOCKS - 1)
    s_ref[...] = jnp.zeros(s_ref.shape, F32)
    issue(start_second, 0, LEAD)
    ax_copy.wait()
    bx_copy.wait()
    wait_for(wq, sems.at[0])
    wait_for(wuk, sems.at[0])
    wait_for(ckv, sems.at[0])
    xa = rows16(ax)

    def absorb(u, _):
        acc = jnp.zeros((16, dc), F32)
        for jj in range(4):
            w_q = head_pair(wq, u, jj)
            w_uk = head_pair(wuk, u, jj)
            for e in range(2):
                q = jnp.dot(xa, w_q[e], preferred_element_type=F32).astype(BF16)
                qa = lax.dot_general(q, w_uk[e], NT, preferred_element_type=F32)
                acc = put_row(2 * jj + e, qa, acc)
            step = u * 4 + jj
            pl.when(step < 8)(lambda: issue(start_second, LEAD + step * 6, 6))
            pl.when(step >= 8)(lambda: issue(start_chunk0, (step - 8) * 3, 3))
        rows = pl.ds(pl.multiple_of(u * 8, 8), 8)
        qa_ref[0, rows, :] = acc[0:8]
        qa_ref[1, rows, :] = acc[8:16]
    lax.fori_loop(0, n_u, absorb, None)

    parts = ckv.shape[0] // 2

    def latent(b, _):
        first_block = 24 + b * 20
        qa = qa_ref[b].astype(BF16)

        def scores(c, _):
            sa_ref[c] = lax.dot_general(qa, ckv[b * parts + c], NT,
                                        preferred_element_type=F32) * sm_scale
            issue(start_chunk0, first_block + 3 * c, 3)
        lax.fori_loop(0, parts, scores, None)

        m = jnp.max(sa_ref[0], axis=1, keepdims=True)
        for c in range(1, parts):
            m = jnp.maximum(m, jnp.max(sa_ref[c], axis=1, keepdims=True))
        l = jnp.zeros_like(m)
        for c in range(parts):
            p = jnp.exp(sa_ref[c] - m)
            l = l + jnp.sum(p, axis=1, keepdims=True)
            pa_ref[c] = p.astype(BF16)

        def context(c, acc):
            acc = acc + jnp.dot(pa_ref[c], ckv[b * parts + c], preferred_element_type=F32)
            issue(start_chunk0, first_block + 12 + 2 * c, 2)
            return acc
        acc = lax.fori_loop(0, parts, context, jnp.zeros((heads, dc), F32)) / l
        rows = pl.ds(pl.multiple_of(b * 8, 8), 8)
        for u in range(n_u):
            cl_ref[u, rows, :] = acc[u * 8:(u + 1) * 8]
    lax.fori_loop(0, 2, latent, None)

    wait_for(bwq, sems.at[1])
    wait_for(wuv, sems.at[1])

    def up_project(u):
        cl = cl_ref[u].astype(BF16)
        acc = jnp.zeros((16, dh), F32)
        for jj in range(4):
            w_uv = head_pair(wuv, u, jj)
            for e in range(2):
                r = jnp.dot(cl, w_uv[e], preferred_element_type=F32)
                acc = put_row(2 * jj + e, r, acc)
        ctx_ref[u] = acc

    def queries(u):
        xb = rows16(bx)
        cols = pl.ds(pl.multiple_of(u * 8 * dh, 8 * dh), 8 * dh)
        k = bwq.shape[1]
        r = sum(jnp.dot(xb[:, n * k:(n + 1) * k], bwq[n, :, cols],
                        preferred_element_type=F32) for n in range(bwq.shape[0]))
        q = jnp.zeros((16, dh), F32)
        for j in range(8):
            q = put_row(j, r[:, j * dh:(j + 1) * dh], q)
        qb_ref[u] = q

    def attend(t, start_next, lead, per_step):
        slot = t % 2
        wait_for(kv.at[slot], sems.at[slot])
        u = t % n_u
        rows = pl.ds(pl.multiple_of((t // n_u) * 8, 8), 8)
        q = qb_ref[u, rows, :].astype(BF16)

        def scores(j, _):
            s = lax.dot_general(q, kv[slot, 0, j], NT, preferred_element_type=F32)
            s_ref[...] = put_row(j, s, s_ref[...])
            issue(start_next, lead + j * per_step, per_step)
        lax.fori_loop(0, G, scores, None)

        s = s_ref[...] * sm_scale
        p = jnp.exp(s - jnp.max(s, axis=1, keepdims=True))
        l = jnp.sum(p, axis=1, keepdims=True)
        p_ref[...] = p.astype(BF16)

        def values(j, acc):
            r = jnp.dot(p_ref[...], kv[slot, 1, j], preferred_element_type=F32)
            issue(start_next, lead + (G + j) * per_step, per_step)
            return put_row(j, r, acc)
        ob_ref[u, rows, :] = lax.fori_loop(0, G, values, jnp.zeros((G, dh), F32)) / l

    def attend_and_fetch(t, _):
        def start_next(i):
            start_chunk(t + 1, i)
        issue(start_next, 0, LEAD)

        @pl.when(t < n_u)
        def _():
            up_project(t)
            queries(t)
        attend(t, start_next, LEAD, (BLOCKS - LEAD) // (2 * G))
    lax.fori_loop(0, n_chunks - 1, attend_and_fetch, None)

    issue(start_last, 0, 24)
    attend(n_chunks - 1, start_last, 24, 2)
    issue(start_tail, 56, 8)
    issue(start_end, 56, 8)

    def head_rows(o_ref, j):
        r = lax.broadcasted_iota(jnp.int32, (8, dh), 0)
        return [
            jnp.where(r == 0,
                      jnp.broadcast_to(o_ref[u, pl.ds(j, 1), :], (8, dh)),
                      jnp.broadcast_to(o_ref[u, pl.ds(8 + j, 1), :], (8, dh))).astype(BF16)
            for u in range(n_u)]

    def add_heads(acc, lhs, w_ref, j, groups):
        rows = pl.ds(pl.multiple_of(j * dh, dh), dh)
        for u in groups:
            acc = acc + jnp.dot(lhs[u], w_ref[u, rows, :], preferred_element_type=F32)
        return acc

    def project(j, accs):
        return (add_heads(accs[0], head_rows(ctx_ref, j), wo, j, range(n_u)),
                add_heads(accs[1], head_rows(ob_ref, j), bwo, j, range(n_u)))

    da = wo.shape[2]
    accs = (jnp.zeros((8, da), F32), jnp.zeros((8, bwo.shape[2]), F32))
    for piece, (lo, hi) in enumerate(((0, SPLIT), (SPLIT, 7))):
        rows = pl.ds(lo * dh, (hi - lo) * dh)
        wait_for(wo.at[:, rows], sems.at[piece])
        wait_for(bwo.at[:, rows], sems.at[piece])
        accs = lax.fori_loop(lo, hi, project, accs)

    rows = pl.ds(7 * dh, dh)
    lhs_a, lhs_b = head_rows(ctx_ref, 7), head_rows(ob_ref, 7)
    wait_for(wo.at[:, rows], sems.at[2])
    wait_for(bwo.at[0:2, rows], sems.at[2])
    acc_a = add_heads(accs[0], lhs_a, wo, 7, range(n_u))
    acc_b = add_heads(accs[1], lhs_b, bwo, 7, (0, 1))
    out_ref[:, :da] = acc_a[0:2].astype(out_ref.dtype)
    wait_for(bwo.at[2:4, rows], sems.at[3])
    acc_b = add_heads(acc_b, lhs_b, bwo, 7, (2, 3))
    out_ref[:, da:] = acc_b[0:2].astype(out_ref.dtype)

    out_copy = pltpu.make_async_copy(out_ref, out_hbm, sems.at[0])
    out_copy.start()
    out_copy.wait()


@jax.jit
def pallas_concat_heads__compressed_kv_cla__gqa_block_cached__decode_kernel(
    A_x: jax.Array,
    A_c_kv: jax.Array,
    A_w_q: jax.Array,
    A_w_uk: jax.Array,
    A_w_uv: jax.Array,
    A_w_o: jax.Array,
    B_x: jax.Array,
    B_k_cache: jax.Array,
    B_v_cache: jax.Array,
    B_wq: jax.Array,
    B_wo: jax.Array,
):
    B, Sq, M = A_x.shape
    _, Sk, Dc = A_c_kv.shape
    _, H, D = A_w_q.shape
    _, Hkv, SkB, Dh = B_k_cache.shape
    MB = B_x.shape[2]
    assert (B, Sq, M, Sk, Dc, H, D) == (2, 1, 512, 4096, 512, 32, 128)
    assert (Hkv, SkB, Dh, MB) == (32, 4096, 128, 512)

    args = (
        A_x.reshape(B, M),
        A_c_kv.reshape(8, B * Sk // 8, Dc),
        A_w_q.reshape(4, M * H // 4, D),
        A_w_uk.reshape(4, Dc * H // 4, D),
        A_w_uv.reshape(4, Dc * H // 4, D),
        A_w_o.reshape(4, H * D // 4, M),
        B_x.reshape(B, MB),
        B_k_cache.reshape(B * Hkv, SkB, Dh),
        B_v_cache.reshape(B * Hkv, SkB, Dh),
        B_wq.reshape(4, MB // 4, Hkv * Dh),
        B_wo.reshape(4, Hkv * Dh // 4, MB),
    )

    def like(x):
        return pltpu.VMEM(x.shape, x.dtype)

    scratch = [
        *(like(x) for x in args[:7]),
        pltpu.VMEM((2, 2, G, SkB, Dh), B_k_cache.dtype),
        like(args[9]),
        like(args[10]),
        pltpu.VMEM((H // 8, 16, Dh), F32),
        pltpu.VMEM((B, H, Dc), F32),
        pltpu.VMEM((4, H, Sk // 4), F32),
        pltpu.VMEM((4, H, Sk // 4), BF16),
        pltpu.VMEM((H // 8, 16, Dc), F32),
        pltpu.VMEM((H // 8, 16, D), F32),
        pltpu.VMEM((H // 8, 16, Dh), F32),
        pltpu.VMEM((G, SkB), F32),
        pltpu.VMEM((G, SkB), BF16),
        pltpu.VMEM((B, M + MB), A_x.dtype),
        pltpu.SemaphoreType.DMA((4,)),
    ]
    out = pl.pallas_call(
        _kernel,
        in_specs=[pl.BlockSpec(memory_space=pltpu.HBM)] * len(args),
        out_specs=pl.BlockSpec(memory_space=pltpu.HBM),
        out_shape=jax.ShapeDtypeStruct((B, M + MB), A_x.dtype),
        scratch_shapes=scratch,
        compiler_params=pltpu.CompilerParams(vmem_limit_bytes=100 * 1024 * 1024),
    )(*args)
    return out.reshape(B, Sq, M + MB)
```

```python
import jax
import jax.numpy as jnp
from jax import lax
import jax.experimental.pallas as pl
import jax.experimental.pallas.tpu as pltpu

F32 = jnp.float32
BF16 = jnp.bfloat16
NT = (((1,), (1,)), ((), ()))

G = 8
BLOCKS = 64
LEAD = 16
SPLIT = 5


def _kernel(ax_hbm, ckv_hbm, wq_hbm, wuk_hbm, wuv_hbm, wo_hbm,
            bx_hbm, k_hbm, v_hbm, bwq_hbm, bwo_hbm,
            out_hbm,
            ax, ckv, w3, wo, bx, kv, bwq, bwo,
            words, by_head, qb_ref, qa_ref, sa_ref, pa_ref, cl_ref, ctx_ref, ob_ref, s_ref, p_ref,
            out_ref, sems):
    n_pairs, _, dh = k_hbm.shape
    n_chunks = n_pairs // G
    wq, wuk, wuv = w3.at[0], w3.at[1], w3.at[2]
    heads = qa_ref.shape[1]
    n_u = heads // 8
    dc = ckv.shape[2]
    sm_scale = dh ** -0.5

    def copy(src, dst, idx, sem, queue):
        pltpu.make_async_copy(src.at[idx], dst.at[idx], sem).start(priority=queue)

    def wait_for(buf, sem):
        pltpu.make_async_copy(buf, buf, sem).wait()

    def start_tall(src, dst, sem, i, pair, queue):
        copy(src, dst, (pl.ds(2 * pair, 2), pl.ds(2 * i, 2)), sem, queue)

    def start_wide(src, dst, sem, i, pair, queue):
        rows = pl.ds(pl.multiple_of(i * 16, 16), 16)
        copy(src, dst, (pl.ds(2 * pair, 2), rows), sem, queue)

    def start_flat(src, dst, sem, i, pair, queue):
        rows = pl.ds(pl.multiple_of((i // 4) * 8, 8), 8)
        cols = pl.ds(pl.multiple_of((i % 4) * 1024, 1024), 1024)
        copy(src, dst, (pl.ds(2 * pair, 2), rows, cols), sem, queue)

    def start_first(i):
        for g, (src, dst) in enumerate(((wq_hbm, wq), (wuk_hbm, wuk))):
            for pair in range(2):
                start_tall(src, dst, sems.at[0], i, pair, 0)
                start_wide(ckv_hbm, ckv, sems.at[0], i, 2 * g + pair, 1)

    def start_second(i):
        for pair in range(2):
            start_flat(bwq_hbm, bwq, sems.at[1], i, pair, 0)
            start_tall(wuv_hbm, wuv, sems.at[1], i, pair, 1)

    def start_chunk(t, i):
        slot = t % 2
        rows = pl.ds(pl.multiple_of(i * 64, 64), 64)
        for pair in range(G // 2):
            for a, src in enumerate((k_hbm, v_hbm)):
                pltpu.make_async_copy(
                    src.at[pl.ds(t * G + 2 * pair, 2), rows],
                    kv.at[slot, a, pl.ds(2 * pair, 2), rows],
                    sems.at[slot],
                ).start(priority=a)

    def start_chunk0(i):
        start_chunk(0, i)

    def start_last(i):
        sem = sems.at[(i >= 8 * SPLIT).astype(jnp.int32)]
        for pair in range(2):
            start_wide(wo_hbm, wo, sem, i, pair, 0)
            start_wide(bwo_hbm, bwo, sem, i, pair, 1)

    def start_tail(i):
        start_wide(wo_hbm, wo, sems.at[2], i, 0, 1)
        start_wide(wo_hbm, wo, sems.at[2], i, 1, 1)
        start_wide(bwo_hbm, bwo, sems.at[2], i, 0, 1)

    def start_end(i):
        start_wide(bwo_hbm, bwo, sems.at[3], i, 1, 1)

    def issue(start, first_block, n_blocks):
        def body(i, _):
            start(first_block + i)
        lax.fori_loop(0, n_blocks, body, None)

    def rows16(x_ref):
        x = x_ref[...].astype(F32)
        shape = (16, x.shape[1])
        r = lax.broadcasted_iota(jnp.int32, shape, 0)
        return jnp.where(r < 8, jnp.broadcast_to(x[0:1], shape),
                         jnp.broadcast_to(x[1:2], shape)).astype(BF16)

    def put_row(j, new, old):
        r = lax.broadcasted_iota(jnp.int32, new.shape, 0)
        return jnp.where((r & 7) == j, new, old)

    def split_heads(which, g, dst, between=lambda k: None):
        n_slabs, m = w3.shape[1:3]

        def to_words(n, _):
            x = w3[which, n, :, pl.ds(pl.multiple_of(16 * g, 16), 16), :]
            words[pl.ds(pl.multiple_of(n * m * 8, m * 8), m * 8), :] = pltpu.bitcast(
                x.reshape(m * 16, dh), jnp.uint32)
        lax.fori_loop(0, n_slabs, to_words, None)
        between(0)
        for e in range(8):
            x = words[pl.ds(e, n_slabs * m, stride=8), :]
            by_head[dst, 2 * e] = pltpu.bitcast(x << 16, F32).astype(BF16)
            by_head[dst, 2 * e + 1] = pltpu.bitcast(
                x & jnp.uint32(0xFFFF0000), F32).astype(BF16)
            if e % 2:
                between(1 + e // 2)

    start_first(0)
    ax_copy = pltpu.make_async_copy(ax_hbm, ax, sems.at[2])
    bx_copy = pltpu.make_async_copy(bx_hbm, bx, sems.at[3])
    ax_copy.start()
    bx_copy.start()
    issue(start_first, 1, BLOCKS - 1)
    s_ref[...] = jnp.zeros(s_ref.shape, F32)
    issue(start_second, 0, LEAD)
    ax_copy.wait()
    bx_copy.wait()
    wait_for(wq, sems.at[0])
    wait_for(wuk, sems.at[0])
    wait_for(ckv, sems.at[0])
    xa = rows16(ax)

    def absorb(g, _):
        def fetch(second, chunk0):
            pl.when(g == 0)(lambda: issue(start_second, *second))
            pl.when(g == 1)(lambda: issue(start_chunk0, *chunk0))

        def split(which, _):
            def between(k):
                first, n = (0, 2) if k == 0 else (k + 1, 1)
                first = which * 6 + first
                fetch((LEAD + 2 * first, 2 * n), (first, n))
            split_heads(which, g, which, between)
        lax.fori_loop(0, 2, split, None)

        def eight_heads(v, _):
            def two_heads(jj, acc):
                for e in range(2):
                    h = v * 8 + 2 * jj + e
                    q = jnp.dot(xa, by_head[0, h], preferred_element_type=F32)
                    qa = lax.dot_general(q.astype(BF16), by_head[1, h], NT,
                                         preferred_element_type=F32)
                    acc = put_row(2 * jj + e, qa, acc)
                step = v * 4 + jj
                fetch((LEAD + 24 + 3 * step, 3), (12 + 2 * step, 2))
                return acc
            acc = lax.fori_loop(0, 4, two_heads, jnp.zeros((16, dc), F32))
            rows = pl.ds(pl.multiple_of((2 * g + v) * 8, 8), 8)
            qa_ref[0, rows, :] = acc[0:8]
            qa_ref[1, rows, :] = acc[8:16]
        lax.fori_loop(0, 2, eight_heads, None)
    lax.fori_loop(0, 2, absorb, None)

    parts = ckv.shape[0] // 2

    def latent(b, _):
        first = 28 + b * 18
        qa = qa_ref[b].astype(BF16)

        def scores(c, _):
            sa_ref[c] = lax.dot_general(qa, ckv[b * parts + c], NT,
                                        preferred_element_type=F32) * sm_scale
            issue(start_chunk0, first + 2 * c, 2)
        lax.fori_loop(0, parts, scores, None)
        issue(start_chunk0, first + 8, 2)

        m = jnp.max(sa_ref[0], axis=1, keepdims=True)
        for c in range(1, parts):
            m = jnp.maximum(m, jnp.max(sa_ref[c], axis=1, keepdims=True))
        l = jnp.zeros_like(m)
        for c in range(parts):
            p = jnp.exp(sa_ref[c] - m)
            l = l + jnp.sum(p, axis=1, keepdims=True)
            pa_ref[c] = p.astype(BF16)

        def context(c, acc):
            acc = acc + jnp.dot(pa_ref[c], ckv[b * parts + c], preferred_element_type=F32)
            issue(start_chunk0, first + 10 + 2 * c, 2)
            return acc
        acc = lax.fori_loop(0, parts, context, jnp.zeros((heads, dc), F32)) / l
        rows = pl.ds(pl.multiple_of(b * 8, 8), 8)
        for u in range(n_u):
            cl_ref[u, rows, :] = acc[u * 8:(u + 1) * 8]
    lax.fori_loop(0, 2, latent, None)

    wait_for(bwq, sems.at[1])
    wait_for(wuv, sems.at[1])

    def up_project(u):
        cl = cl_ref[u].astype(BF16)

        def one_head(j, acc):
            r = jnp.dot(cl, by_head[u // 2, (u % 2) * 8 + j], preferred_element_type=F32)
            return put_row(j, r, acc)
        ctx_ref[u] = lax.fori_loop(0, 8, one_head, jnp.zeros((16, dh), F32))

    def queries(u):
        xb = rows16(bx)
        cols = pl.ds(pl.multiple_of(u * 8 * dh, 8 * dh), 8 * dh)
        k = bwq.shape[1]
        r = sum(jnp.dot(xb[:, n * k:(n + 1) * k], bwq[n, :, cols],
                        preferred_element_type=F32) for n in range(bwq.shape[0]))
        q = jnp.zeros((16, dh), F32)
        for j in range(8):
            q = put_row(j, r[:, j * dh:(j + 1) * dh], q)
        qb_ref[u] = q

    def attend(t, start_next, lead, per_step):
        slot = t % 2
        wait_for(kv.at[slot], sems.at[slot])
        u = t % n_u
        rows = pl.ds(pl.multiple_of((t // n_u) * 8, 8), 8)
        q = qb_ref[u, rows, :].astype(BF16)

        def scores(j, _):
            s = lax.dot_general(q, kv[slot, 0, j], NT, preferred_element_type=F32)
            s_ref[...] = put_row(j, s, s_ref[...])
            issue(start_next, lead + j * per_step, per_step)
        lax.fori_loop(0, G, scores, None)

        s = s_ref[...] * sm_scale
        p = jnp.exp(s - jnp.max(s, axis=1, keepdims=True))
        l = jnp.sum(p, axis=1, keepdims=True)
        p_ref[...] = p.astype(BF16)

        def values(j, acc):
            r = jnp.dot(p_ref[...], kv[slot, 1, j], preferred_element_type=F32)
            issue(start_next, lead + (G + j) * per_step, per_step)
            return put_row(j, r, acc)
        ob_ref[u, rows, :] = lax.fori_loop(0, G, values, jnp.zeros((G, dh), F32)) / l

    def attend_and_fetch(t, _):
        def start_next(i):
            start_chunk(t + 1, i)
        issue(start_next, 0, LEAD)

        pl.when(t < n_u)(lambda: queries(t))
        pl.when(t < 2)(lambda: split_heads(2, t, t))
        pl.when((t >= 2) & (t < 2 + n_u))(lambda: up_project(t - 2))
        attend(t, start_next, LEAD, (BLOCKS - LEAD) // (2 * G))
    lax.fori_loop(0, n_chunks - 1, attend_and_fetch, None)

    issue(start_last, 0, 24)
    attend(n_chunks - 1, start_last, 24, 2)
    issue(start_tail, 56, 8)
    issue(start_end, 56, 8)

    def head_rows(o_ref, j):
        r = lax.broadcasted_iota(jnp.int32, (8, dh), 0)
        return [
            jnp.where(r == 0,
                      jnp.broadcast_to(o_ref[u, pl.ds(j, 1), :], (8, dh)),
                      jnp.broadcast_to(o_ref[u, pl.ds(8 + j, 1), :], (8, dh))).astype(BF16)
            for u in range(n_u)]

    def add_heads(acc, lhs, w_ref, j, groups):
        rows = pl.ds(pl.multiple_of(j * dh, dh), dh)
        for u in groups:
            acc = acc + jnp.dot(lhs[u], w_ref[u, rows, :], preferred_element_type=F32)
        return acc

    def project(j, accs):
        return (add_heads(accs[0], head_rows(ctx_ref, j), wo, j, range(n_u)),
                add_heads(accs[1], head_rows(ob_ref, j), bwo, j, range(n_u)))

    da = wo.shape[2]
    accs = (jnp.zeros((8, da), F32), jnp.zeros((8, bwo.shape[2]), F32))
    for piece, (lo, hi) in enumerate(((0, SPLIT), (SPLIT, 7))):
        rows = pl.ds(lo * dh, (hi - lo) * dh)
        wait_for(wo.at[:, rows], sems.at[piece])
        wait_for(bwo.at[:, rows], sems.at[piece])
        accs = lax.fori_loop(lo, hi, project, accs)

    rows = pl.ds(7 * dh, dh)
    lhs_a, lhs_b = head_rows(ctx_ref, 7), head_rows(ob_ref, 7)
    wait_for(wo.at[:, rows], sems.at[2])
    wait_for(bwo.at[0:2, rows], sems.at[2])
    acc_a = add_heads(accs[0], lhs_a, wo, 7, range(n_u))
    acc_b = add_heads(accs[1], lhs_b, bwo, 7, (0, 1))
    out_ref[:, :da] = acc_a[0:2].astype(out_ref.dtype)
    wait_for(bwo.at[2:4, rows], sems.at[3])
    acc_b = add_heads(acc_b, lhs_b, bwo, 7, (2, 3))
    out_ref[:, da:] = acc_b[0:2].astype(out_ref.dtype)

    out_copy = pltpu.make_async_copy(out_ref, out_hbm, sems.at[0])
    out_copy.start()
    out_copy.wait()


@jax.jit
def pallas_concat_heads__compressed_kv_cla__gqa_block_cached__decode_kernel(
    A_x: jax.Array,
    A_c_kv: jax.Array,
    A_w_q: jax.Array,
    A_w_uk: jax.Array,
    A_w_uv: jax.Array,
    A_w_o: jax.Array,
    B_x: jax.Array,
    B_k_cache: jax.Array,
    B_v_cache: jax.Array,
    B_wq: jax.Array,
    B_wo: jax.Array,
):
    B, Sq, M = A_x.shape
    _, Sk, Dc = A_c_kv.shape
    _, H, D = A_w_q.shape
    _, Hkv, SkB, Dh = B_k_cache.shape
    MB = B_x.shape[2]
    assert (B, Sq, M, Sk, Dc, H, D) == (2, 1, 512, 4096, 512, 32, 128)
    assert (Hkv, SkB, Dh, MB) == (32, 4096, 128, 512)

    args = (
        A_x.reshape(B, M),
        A_c_kv.reshape(8, B * Sk // 8, Dc),
        A_w_q.reshape(4, M // 4, H, D),
        A_w_uk.reshape(4, Dc // 4, H, D),
        A_w_uv.reshape(4, Dc // 4, H, D),
        A_w_o.reshape(4, H * D // 4, M),
        B_x.reshape(B, MB),
        B_k_cache.reshape(B * Hkv, SkB, Dh),
        B_v_cache.reshape(B * Hkv, SkB, Dh),
        B_wq.reshape(4, MB // 4, Hkv * Dh),
        B_wo.reshape(4, Hkv * Dh // 4, MB),
    )

    def like(x):
        return pltpu.VMEM(x.shape, x.dtype)

    scratch = [
        like(args[0]),
        like(args[1]),
        pltpu.VMEM((3, *args[2].shape), BF16),
        like(args[5]),
        like(args[6]),
        pltpu.VMEM((2, 2, G, SkB, Dh), B_k_cache.dtype),
        like(args[9]),
        like(args[10]),
        pltpu.VMEM((M * 8, D), jnp.uint32),
        pltpu.VMEM((2, 16, M, D), BF16),
        pltpu.VMEM((H // 8, 16, Dh), F32),
        pltpu.VMEM((B, H, Dc), F32),
        pltpu.VMEM((4, H, Sk // 4), F32),
        pltpu.VMEM((4, H, Sk // 4), BF16),
        pltpu.VMEM((H // 8, 16, Dc), F32),
        pltpu.VMEM((H // 8, 16, D), F32),
        pltpu.VMEM((H // 8, 16, Dh), F32),
        pltpu.VMEM((G, SkB), F32),
        pltpu.VMEM((G, SkB), BF16),
        pltpu.VMEM((B, M + MB), A_x.dtype),
        pltpu.SemaphoreType.DMA((4,)),
    ]
    out = pl.pallas_call(
        _kernel,
        in_specs=[pl.BlockSpec(memory_space=pltpu.HBM)] * len(args),
        out_specs=pl.BlockSpec(memory_space=pltpu.HBM),
        out_shape=jax.ShapeDtypeStruct((B, M + MB), A_x.dtype),
        scratch_shapes=scratch,
        compiler_params=pltpu.CompilerParams(vmem_limit_bytes=100 * 1024 * 1024),
    )(*args)
    return out.reshape(B, Sq, M + MB)
```

```python
import jax
import jax.numpy as jnp
from jax import lax
import jax.experimental.pallas as pl
import jax.experimental.pallas.tpu as pltpu

F32 = jnp.float32
BF16 = jnp.bfloat16
NT = (((1,), (1,)), ((), ()))

G = 8
BLOCKS = 64
LEAD = 16
SPLIT = 5


def _kernel(ax_hbm, ckv_hbm, wq_hbm, wuk_hbm, wuv_hbm, wo_hbm,
            bx_hbm, k_hbm, v_hbm, bwq_hbm, bwo_hbm,
            out_hbm,
            ax, bx, ckv, w3, bwq, w_out, kv,
            words, by_head, qb_ref, qa_ref, sa_ref, pa_ref, cl_ref, ctx_ref, ob_ref, s_ref, p_ref,
            out_ref, sems):
    n_pairs, _, dh = k_hbm.shape
    n_chunks = n_pairs // G
    wq, wuk, wuv = w3.at[0], w3.at[1], w3.at[2]
    wo, bwo = w_out.at[0:4], w_out.at[4:8]
    heads = qa_ref.shape[1]
    n_u = heads // 8
    dc = ckv.shape[2]
    sm_scale = dh ** -0.5

    def copy(src, dst, idx, sem, queue):
        pltpu.make_async_copy(src.at[idx], dst.at[idx], sem).start(priority=queue)

    def wait_for(buf, sem):
        pltpu.make_async_copy(buf, buf, sem).wait()

    def start_tall(src, dst, sem, i, pair, queue):
        copy(src, dst, (pl.ds(2 * pair, 2), pl.ds(2 * i, 2)), sem, queue)

    def start_wide(src, dst, sem, i, pair, queue):
        rows = pl.ds(pl.multiple_of(i * 16, 16), 16)
        copy(src, dst, (pl.ds(2 * pair, 2), rows), sem, queue)

    def start_flat(src, dst, sem, i, pair, queue):
        rows = pl.ds(pl.multiple_of((i // 4) * 8, 8), 8)
        cols = pl.ds(pl.multiple_of((i % 4) * 1024, 1024), 1024)
        copy(src, dst, (pl.ds(2 * pair, 2), rows, cols), sem, queue)

    def start_first(i):
        for g, (src, dst) in enumerate(((wq_hbm, wq), (wuk_hbm, wuk))):
            for pair in range(2):
                start_tall(src, dst, sems.at[0], i, pair, 0)
                start_wide(ckv_hbm, ckv, sems.at[1], i, 2 * g + pair, 1)

    def start_second(i):
        for pair in range(2):
            start_flat(bwq_hbm, bwq, sems.at[2], i, pair, 0)
            start_tall(wuv_hbm, wuv, sems.at[3], i, pair, 1)

    def start_chunk(t, i):
        slot = t % 2
        rows = pl.ds(pl.multiple_of(i * 64, 64), 64)
        for pair in range(G // 2):
            for a, src in enumerate((k_hbm, v_hbm)):
                pltpu.make_async_copy(
                    src.at[pl.ds(t * G + 2 * pair, 2), rows],
                    kv.at[slot, a, pl.ds(2 * pair, 2), rows],
                    sems.at[slot],
                ).start(priority=a)

    def start_chunk0(i):
        start_chunk(0, i)

    def start_last(i):
        sem = sems.at[(i >= 8 * SPLIT).astype(jnp.int32)]
        for pair in range(2):
            start_wide(wo_hbm, wo, sem, i, pair, 0)
            start_wide(bwo_hbm, bwo, sem, i, pair, 1)

    def start_tail(i):
        start_wide(wo_hbm, wo, sems.at[2], i, 0, 1)
        start_wide(wo_hbm, wo, sems.at[2], i, 1, 1)
        start_wide(bwo_hbm, bwo, sems.at[2], i, 0, 1)

    def start_end(i):
        start_wide(bwo_hbm, bwo, sems.at[3], i, 1, 1)

    def issue(start, first_block, n_blocks):
        def body(i, _):
            start(first_block + i)
        lax.fori_loop(0, n_blocks, body, None)

    def rows16(x_ref):
        x = x_ref[...].astype(F32)
        shape = (16, x.shape[1])
        r = lax.broadcasted_iota(jnp.int32, shape, 0)
        return jnp.where(r < 8, jnp.broadcast_to(x[0:1], shape),
                         jnp.broadcast_to(x[1:2], shape)).astype(BF16)

    def put_row(j, new, old):
        r = lax.broadcasted_iota(jnp.int32, new.shape, 0)
        return jnp.where((r & 7) == j, new, old)

    def split_heads(which, g, dst, between=lambda k: None):
        n_slabs, m = w3.shape[1:3]

        def to_words(n, _):
            x = w3[which, n, :, pl.ds(pl.multiple_of(16 * g, 16), 16), :]
            words[pl.ds(pl.multiple_of(n * m * 8, m * 8), m * 8), :] = pltpu.bitcast(
                x.reshape(m * 16, dh), jnp.uint32)
        lax.fori_loop(0, n_slabs, to_words, None)
        between(0)
        for e in range(8):
            x = words[pl.ds(e, n_slabs * m, stride=8), :]
            by_head[dst, 2 * e] = pltpu.bitcast(x << 16, F32).astype(BF16)
            by_head[dst, 2 * e + 1] = pltpu.bitcast(
                x & jnp.uint32(0xFFFF0000), F32).astype(BF16)
            if e % 2:
                between(1 + e // 2)

    start_first(0)
    ax_copy = pltpu.make_async_copy(ax_hbm, ax, sems.at[2])
    bx_copy = pltpu.make_async_copy(bx_hbm, bx, sems.at[3])
    ax_copy.start()
    bx_copy.start()
    issue(start_first, 1, BLOCKS - 1)
    s_ref[...] = jnp.zeros(s_ref.shape, F32)
    ax_copy.wait()
    bx_copy.wait()
    issue(start_second, 0, LEAD)
    wait_for(w3.at[0:2], sems.at[0])
    wait_for(ckv, sems.at[1])
    xa = rows16(ax)

    def absorb(g, _):
        def fetch(second, chunk0):
            pl.when(g == 0)(lambda: issue(start_second, *second))
            pl.when(g == 1)(lambda: issue(start_chunk0, *chunk0))

        def split(which, _):
            def between(k):
                first, n = (0, 2) if k == 0 else (k + 1, 1)
                first = which * 6 + first
                fetch((LEAD + 2 * first, 2 * n), (first, n))
            split_heads(which, g, which, between)
        lax.fori_loop(0, 2, split, None)

        def eight_heads(v, _):
            def two_heads(jj, acc):
                for e in range(2):
                    h = v * 8 + 2 * jj + e
                    q = jnp.dot(xa, by_head[0, h], preferred_element_type=F32)
                    qa = lax.dot_general(q.astype(BF16), by_head[1, h], NT,
                                         preferred_element_type=F32)
                    acc = put_row(2 * jj + e, qa, acc)
                step = v * 4 + jj
                fetch((LEAD + 24 + 3 * step, 3), (12 + 2 * step, 2))
                return acc
            acc = lax.fori_loop(0, 4, two_heads, jnp.zeros((16, dc), F32))
            rows = pl.ds(pl.multiple_of((2 * g + v) * 8, 8), 8)
            qa_ref[0, rows, :] = acc[0:8]
            qa_ref[1, rows, :] = acc[8:16]
        lax.fori_loop(0, 2, eight_heads, None)
    lax.fori_loop(0, 2, absorb, None)

    parts = ckv.shape[0] // 2

    def latent(b, _):
        first = 28 + b * 18
        qa = qa_ref[b].astype(BF16)

        def scores(c, _):
            sa_ref[c] = lax.dot_general(qa, ckv[b * parts + c], NT,
                                        preferred_element_type=F32) * sm_scale
            issue(start_chunk0, first + 2 * c, 2)
        lax.fori_loop(0, parts, scores, None)
        issue(start_chunk0, first + 8, 2)

        m = jnp.max(sa_ref[0], axis=1, keepdims=True)
        for c in range(1, parts):
            m = jnp.maximum(m, jnp.max(sa_ref[c], axis=1, keepdims=True))
        l = jnp.zeros_like(m)
        for c in range(parts):
            p = jnp.exp(sa_ref[c] - m)
            l = l + jnp.sum(p, axis=1, keepdims=True)
            pa_ref[c] = p.astype(BF16)

        def context(c, acc):
            acc = acc + jnp.dot(pa_ref[c], ckv[b * parts + c], preferred_element_type=F32)
            issue(start_chunk0, first + 10 + 2 * c, 2)
            return acc
        acc = lax.fori_loop(0, parts, context, jnp.zeros((heads, dc), F32)) / l
        rows = pl.ds(pl.multiple_of(b * 8, 8), 8)
        for u in range(n_u):
            cl_ref[u, rows, :] = acc[u * 8:(u + 1) * 8]
    lax.fori_loop(0, 2, latent, None)

    wait_for(bwq, sems.at[2])
    wait_for(wuv, sems.at[3])

    def up_project(u):
        cl = cl_ref[u].astype(BF16)

        def one_head(j, acc):
            r = jnp.dot(cl, by_head[u // 2, (u % 2) * 8 + j], preferred_element_type=F32)
            return put_row(j, r, acc)
        ctx_ref[u] = lax.fori_loop(0, 8, one_head, jnp.zeros((16, dh), F32))

    def queries(u):
        xb = rows16(bx)
        cols = pl.ds(pl.multiple_of(u * 8 * dh, 8 * dh), 8 * dh)
        k = bwq.shape[1]
        r = sum(jnp.dot(xb[:, n * k:(n + 1) * k], bwq[n, :, cols],
                        preferred_element_type=F32) for n in range(bwq.shape[0]))
        q = jnp.zeros((16, dh), F32)
        for j in range(8):
            q = put_row(j, r[:, j * dh:(j + 1) * dh], q)
        qb_ref[u] = q

    def attend(t, start_next, lead, per_step):
        slot = t % 2
        wait_for(kv.at[slot], sems.at[slot])
        u = t % n_u
        rows = pl.ds(pl.multiple_of((t // n_u) * 8, 8), 8)
        q = qb_ref[u, rows, :].astype(BF16)

        def scores(j, _):
            s = lax.dot_general(q, kv[slot, 0, j], NT, preferred_element_type=F32)
            s_ref[...] = put_row(j, s, s_ref[...])
            issue(start_next, lead + j * per_step, per_step)
        lax.fori_loop(0, G, scores, None)

        s = s_ref[...] * sm_scale
        p = jnp.exp(s - jnp.max(s, axis=1, keepdims=True))
        l = jnp.sum(p, axis=1, keepdims=True)
        p_ref[...] = p.astype(BF16)

        def values(j, acc):
            r = jnp.dot(p_ref[...], kv[slot, 1, j], preferred_element_type=F32)
            issue(start_next, lead + (G + j) * per_step, per_step)
            return put_row(j, r, acc)
        ob_ref[u, rows, :] = lax.fori_loop(0, G, values, jnp.zeros((G, dh), F32)) / l

    def attend_and_fetch(t, _):
        def start_next(i):
            start_chunk(t + 1, i)
        issue(start_next, 0, LEAD)

        pl.when(t < n_u)(lambda: queries(t))
        pl.when(t < 2)(lambda: split_heads(2, t, t))
        pl.when((t >= 2) & (t < 2 + n_u))(lambda: up_project(t - 2))
        attend(t, start_next, LEAD, (BLOCKS - LEAD) // (2 * G))
    lax.fori_loop(0, n_chunks - 1, attend_and_fetch, None)

    issue(start_last, 0, 24)
    attend(n_chunks - 1, start_last, 24, 2)
    issue(start_tail, 56, 8)
    issue(start_end, 56, 8)

    def head_rows(o_ref, j):
        r = lax.broadcasted_iota(jnp.int32, (8, dh), 0)
        return [
            jnp.where(r == 0,
                      jnp.broadcast_to(o_ref[u, pl.ds(j, 1), :], (8, dh)),
                      jnp.broadcast_to(o_ref[u, pl.ds(8 + j, 1), :], (8, dh))).astype(BF16)
            for u in range(n_u)]

    def add_heads(acc, lhs, first_slab, j, groups):
        rows = pl.ds(pl.multiple_of(j * dh, dh), dh)
        for u in groups:
            acc = acc + jnp.dot(lhs[u], w_out[first_slab + u, rows, :],
                                preferred_element_type=F32)
        return acc

    def project(j, accs):
        return (add_heads(accs[0], head_rows(ctx_ref, j), 0, j, range(n_u)),
                add_heads(accs[1], head_rows(ob_ref, j), n_u, j, range(n_u)))

    dm = w_out.shape[2]
    accs = (jnp.zeros((8, dm), F32), jnp.zeros((8, dm), F32))
    for piece, (lo, hi) in enumerate(((0, SPLIT), (SPLIT, 7))):
        wait_for(w_out.at[:, pl.ds(lo * dh, (hi - lo) * dh)], sems.at[piece])
        accs = lax.fori_loop(lo, hi, project, accs)

    rows = pl.ds(7 * dh, dh)
    lhs_a, lhs_b = head_rows(ctx_ref, 7), head_rows(ob_ref, 7)
    wait_for(w_out.at[0:6, rows], sems.at[2])
    acc_a = add_heads(accs[0], lhs_a, 0, 7, range(n_u))
    acc_b = add_heads(accs[1], lhs_b, n_u, 7, (0, 1))
    out_ref[:, :dm] = acc_a[0:2].astype(out_ref.dtype)
    wait_for(w_out.at[6:8, rows], sems.at[3])
    acc_b = add_heads(acc_b, lhs_b, n_u, 7, (2, 3))
    out_ref[:, dm:] = acc_b[0:2].astype(out_ref.dtype)

    out_copy = pltpu.make_async_copy(out_ref, out_hbm, sems.at[0])
    out_copy.start()
    out_copy.wait()


@jax.jit
def pallas_concat_heads__compressed_kv_cla__gqa_block_cached__decode_kernel(
    A_x: jax.Array,
    A_c_kv: jax.Array,
    A_w_q: jax.Array,
    A_w_uk: jax.Array,
    A_w_uv: jax.Array,
    A_w_o: jax.Array,
    B_x: jax.Array,
    B_k_cache: jax.Array,
    B_v_cache: jax.Array,
    B_wq: jax.Array,
    B_wo: jax.Array,
):
    B, Sq, M = A_x.shape
    _, Sk, Dc = A_c_kv.shape
    _, H, D = A_w_q.shape
    _, Hkv, SkB, Dh = B_k_cache.shape
    MB = B_x.shape[2]
    assert (B, Sq, M, Sk, Dc, H, D) == (2, 1, 512, 4096, 512, 32, 128)
    assert (Hkv, SkB, Dh, MB) == (32, 4096, 128, 512)

    args = (
        A_x.reshape(B, M),
        A_c_kv.reshape(8, B * Sk // 8, Dc),
        A_w_q.reshape(4, M // 4, H, D),
        A_w_uk.reshape(4, Dc // 4, H, D),
        A_w_uv.reshape(4, Dc // 4, H, D),
        A_w_o.reshape(4, H * D // 4, M),
        B_x.reshape(B, MB),
        B_k_cache.reshape(B * Hkv, SkB, Dh),
        B_v_cache.reshape(B * Hkv, SkB, Dh),
        B_wq.reshape(4, MB // 4, Hkv * Dh),
        B_wo.reshape(4, Hkv * Dh // 4, MB),
    )

    def like(x):
        return pltpu.VMEM(x.shape, x.dtype)

    scratch = [
        like(args[0]),
        like(args[6]),
        like(args[1]),
        pltpu.VMEM((3, *args[2].shape), BF16),
        like(args[9]),
        pltpu.VMEM((8, H * D // 4, M), BF16),
        pltpu.VMEM((2, 2, G, SkB, Dh), BF16),
        pltpu.VMEM((M * 8, D), jnp.uint32),
        pltpu.VMEM((2, 16, M, D), BF16),
        pltpu.VMEM((H // 8, 16, Dh), F32),
        pltpu.VMEM((B, H, Dc), F32),
        pltpu.VMEM((4, H, Sk // 4), F32),
        pltpu.VMEM((4, H, Sk // 4), BF16),
        pltpu.VMEM((H // 8, 16, Dc), F32),
        pltpu.VMEM((H // 8, 16, D), F32),
        pltpu.VMEM((H // 8, 16, Dh), F32),
        pltpu.VMEM((G, SkB), F32),
        pltpu.VMEM((G, SkB), BF16),
        pltpu.VMEM((B, M + MB), A_x.dtype),
        pltpu.SemaphoreType.DMA((4,)),
    ]
    out = pl.pallas_call(
        _kernel,
        in_specs=[pl.BlockSpec(memory_space=pltpu.HBM)] * len(args),
        out_specs=pl.BlockSpec(memory_space=pltpu.HBM),
        out_shape=jax.ShapeDtypeStruct((B, M + MB), A_x.dtype),
        scratch_shapes=scratch,
        compiler_params=pltpu.CompilerParams(vmem_limit_bytes=100 * 1024 * 1024),
    )(*args)
    return out.reshape(B, Sq, M + MB)
```
